```python
import os as _os
_os.environ.setdefault("JAX_PLATFORMS", "cpu")
import jax
import jax.numpy as jnp

def _softmax(x, axis=-1):
    return jax.nn.softmax(x, axis=axis)
def _gelu(x):
    return jax.nn.gelu(x, approximate=True)
def _silu(x):
    return jax.nn.silu(x)
def _sigmoid(x):
    return jax.nn.sigmoid(x)
def _layernorm(x, axis=-1, eps=1e-5):
    m = jnp.mean(x, axis=axis, keepdims=True)
    v = jnp.var(x, axis=axis, keepdims=True)
    return (x - m) / jnp.sqrt(v + eps)
def _scatter_add(tgt, idx, src, axis=0):
    return tgt.at[idx].add(src)
def _segment_sum(src, seg, n):
    return jax.ops.segment_sum(src, seg, n)
class _Rng:
    def __init__(self, key):
        self._k = key
    def _next(self):
        self._k, sub = jax.random.split(self._k)
        return sub
    def normal(self, shape):
        return jax.random.normal(self._next(), shape, dtype=jnp.bfloat16)
    def randint(self, lo, hi, shape):
        return jax.random.randint(self._next(), shape, lo, hi, dtype=jnp.int32)
    def uniform(self, shape, lo=0.0, hi=1.0):
        return jax.random.uniform(self._next(), shape, jnp.bfloat16, lo, hi)
    def permutation(self, n):
        return jax.random.permutation(self._next(), n)


kernel_name = 'standalone__instancenorm__sampling'

def setup_inputs():
    _rng = _Rng(jax.random.key(int.from_bytes(__import__("os").urandom(4), "little")))
    _w = (lambda a: (lambda t: t.astype(jnp.bfloat16) if jnp.issubdtype(t.dtype, jnp.floating) else t)(jnp.asarray(a)))
    B, C, H, W = 16, 640, 16, 32
    return {
        "x": _w((lambda *s: _rng.normal(s) * 0.05)(B, C, H, W)),
        "g": _w((lambda *s: _rng.normal(s) * 0.05)(C) + 1.0),
        "b": _w((lambda *s: _rng.normal(s) * 0.05)(C)),
    }

def reference(x, g, b):
    mu = x.mean(axis=(-2, -1), keepdims=True)
    var = ((x - mu) * (x - mu)).mean(axis=(-2, -1), keepdims=True)
    xhat = (x - mu) / jnp.sqrt(var + 1e-5)
    return xhat * g.reshape(1, -1, 1, 1) + b.reshape(1, -1, 1, 1)
```

```python
import jax
import jax.numpy as jnp
import jax.experimental.pallas as pl
import jax.experimental.pallas.tpu as pltpu


def _kernel(x_ref, g_ref, b_ref, o_ref):
    x = x_ref[0].astype(jnp.float32)
    n = x.shape[0]
    mu = jnp.sum(x, axis=0, keepdims=True) * (1.0 / n)
    xc = x - mu
    var = jnp.sum(xc * xc, axis=0, keepdims=True) * (1.0 / n)
    scale = jax.lax.rsqrt(var + 1e-5) * g_ref[...].astype(jnp.float32)
    o_ref[0] = (xc * scale + b_ref[...].astype(jnp.float32)).astype(o_ref.dtype)


@jax.jit
def pallas_standalone__instancenorm__sampling_kernel(
    x: jax.Array,
    g: jax.Array,
    b: jax.Array,
):
    B, C, H, W = x.shape
    HW = H * W
    xt = jnp.transpose(x, (0, 2, 3, 1)).reshape(B, HW, C)
    g2 = g.reshape(1, C)
    b2 = b.reshape(1, C)
    out = pl.pallas_call(
        _kernel,
        grid=(B,),
        in_specs=[
            pl.BlockSpec((1, HW, C), lambda i: (i, 0, 0)),
            pl.BlockSpec((1, C), lambda i: (0, 0)),
            pl.BlockSpec((1, C), lambda i: (0, 0)),
        ],
        out_specs=pl.BlockSpec((1, HW, C), lambda i: (i, 0, 0)),
        out_shape=jax.ShapeDtypeStruct((B, HW, C), x.dtype),
        compiler_params=pltpu.CompilerParams(dimension_semantics=("parallel",)),
    )(xt, g2, b2)
    return jnp.transpose(out.reshape(B, H, W, C), (0, 3, 1, 2))
```

```python
import functools

import jax
import jax.numpy as jnp
import jax.experimental.pallas as pl
import jax.experimental.pallas.tpu as pltpu

_EPS = 1e-5
_LANES = 128


def _schedule(nb):
    if nb >= 16:
        read_chunks = [1, 1, 2, 4]
    elif nb >= 4:
        read_chunks = [1, 1]
    else:
        read_chunks = []
    rest = nb - sum(read_chunks)
    write_groups = []
    while rest > 0:
        n = min(4, rest)
        write_groups.append(n)
        rest -= n
    return read_chunks, write_groups


def _kernel(x_hbm, g_hbm, b_hbm, o_hbm, xbuf, obuf, gbuf, bbuf, rsem, wsem, psem,
            *, nb, read_chunks, write_groups, tail):
    rows, chans = x_hbm.shape
    hw = rows // nb
    ng = chans // _LANES
    kc = sum(read_chunks)

    bounds = [0]
    for n in read_chunks:
        bounds.append(bounds[-1] + n * hw)
    bounds += [rows - tail, rows]
    rds = [
        pltpu.make_async_copy(
            x_hbm.at[pl.ds(a, e - a)], xbuf.at[pl.ds(a, e - a)], rsem.at[n])
        for n, (a, e) in enumerate(zip(bounds[:-1], bounds[1:]))
    ]
    wb = [0, kc] if kc else [0]
    for n in write_groups:
        wb.append(wb[-1] + n)
    wrs = [
        pltpu.make_async_copy(
            obuf.at[pl.ds(a * hw, (e - a) * hw)],
            o_hbm.at[pl.ds(a * hw, (e - a) * hw)],
            wsem.at[n])
        for n, (a, e) in enumerate(zip(wb[:-1], wb[1:]))
    ]
    gcp = pltpu.make_async_copy(g_hbm, gbuf, psem.at[0])
    bcp = pltpu.make_async_copy(b_hbm, bbuf, psem.at[1])

    pre, post = {}, {}
    gcp.start()
    bcp.start()
    started = 0
    while started < min(2, len(rds)):
        rds[started].start()
        started += 1
    first = 0
    for n, cnt in enumerate(read_chunks):
        ev = [rds[n].wait]
        if started < len(rds):
            ev.append(rds[started].start)
            started += 1
        pre[first] = ev
        first += cnt
    assert started == len(rds)
    pre[kc] = [rds[-2].wait] + ([wrs[0].start] if kc else []) + [rds[-1].wait]
    pre[0] = pre[0] + [gcp.wait, bcp.wait]
    for n in range(1 if kc else 0, len(wrs)):
        post[wb[n + 1] - 1] = [wrs[n].start]

    def run_events(table, i):
        for k, ev in table.items():
            @pl.when(i == k)
            def _(ev=ev):
                for act in ev:
                    act()

    def body(i, carry):
        run_events(pre, i)
        s = pl.multiple_of(i * hw, hw)
        for j in range(ng):
            cols = pl.ds(j * _LANES, _LANES)
            x = xbuf[pl.ds(s, hw), cols].astype(jnp.float32)
            mu = jnp.sum(x, axis=0, keepdims=True) * (1.0 / hw)
            xc = x - mu
            var = jnp.sum(xc * xc, axis=0, keepdims=True) * (1.0 / hw)
            scale = jax.lax.rsqrt(var + _EPS) * gbuf[j:j + 1, :].astype(jnp.float32)
            y = xc * scale + bbuf[j:j + 1, :].astype(jnp.float32)
            obuf[pl.ds(s, hw), cols] = y.astype(obuf.dtype)
        run_events(post, i)
        return carry

    jax.lax.fori_loop(0, nb, body, 0)
    for w in wrs:
        w.wait()


@jax.jit
def pallas_standalone__instancenorm__sampling_kernel(
    x: jax.Array,
    g: jax.Array,
    b: jax.Array,
):
    B, C, H, W = x.shape
    HW = H * W
    assert C % _LANES == 0 and HW % 32 == 0
    read_chunks, write_groups = _schedule(B)
    tail = HW // 2

    xt = jnp.transpose(x, (0, 2, 3, 1)).reshape(B * HW, C)
    g2 = g.reshape(C // _LANES, _LANES)
    b2 = b.reshape(C // _LANES, _LANES)

    n_wr = len(write_groups) + (1 if read_chunks else 0)
    out = pl.pallas_call(
        functools.partial(_kernel, nb=B, read_chunks=tuple(read_chunks),
                          write_groups=tuple(write_groups), tail=tail),
        in_specs=[pl.BlockSpec(memory_space=pl.ANY)] * 3,
        out_specs=pl.BlockSpec(memory_space=pl.ANY),
        out_shape=jax.ShapeDtypeStruct((B * HW, C), x.dtype),
        scratch_shapes=[
            pltpu.VMEM((B * HW, C), x.dtype),
            pltpu.VMEM((B * HW, C), x.dtype),
            pltpu.VMEM((C // _LANES, _LANES), g.dtype),
            pltpu.VMEM((C // _LANES, _LANES), b.dtype),
            pltpu.SemaphoreType.DMA((len(read_chunks) + 2,)),
            pltpu.SemaphoreType.DMA((n_wr,)),
            pltpu.SemaphoreType.DMA((2,)),
        ],
        compiler_params=pltpu.CompilerParams(vmem_limit_bytes=48 * 1024 * 1024),
    )(xt, g2, b2)
    return jnp.transpose(out.reshape(B, H, W, C), (0, 3, 1, 2))
```

```python
import functools

import jax
import jax.numpy as jnp
import jax.experimental.pallas as pl
import jax.experimental.pallas.tpu as pltpu

_EPS = 1e-5
_LANES = 128
_PIECE = 16


def _read_chunks(n_stream):
    chunks, size = [], 1
    while sum(chunks) < n_stream:
        chunks.append(min(size, n_stream - sum(chunks)))
        if len(chunks) >= 2:
            size = min(2 * size, 4)
    return tuple(chunks)


def _kernel(x_hbm, g_hbm, b_hbm, o_hbm, xbuf, obuf, gbuf, bbuf, rsem, wsem,
            *, read_chunks, tail):
    nb, hw, chans = o_hbm.shape
    rows = nb * hw
    ng = chans // _LANES
    kc = sum(read_chunks)

    bounds = [0]
    for n in read_chunks:
        bounds.append(bounds[-1] + n * hw)
    bounds += [rows - tail, rows]
    rds = [
        pltpu.make_async_copy(
            x_hbm.at[pl.ds(a, e - a)], xbuf.at[pl.ds(a, e - a)], rsem.at[n % 2])
        for n, (a, e) in enumerate(zip(bounds[:-1], bounds[1:]))
    ]

    def out_copies(lo, hi):
        cps = []
        for r in range(0, hw, _PIECE):
            sl = (pl.ds(lo, hi - lo), pl.ds(r, min(_PIECE, hw - r)), slice(None))
            cps.append(pltpu.make_async_copy(obuf.at[sl], o_hbm.at[sl], wsem.at[0]))
        return cps

    wr_first = out_copies(0, kc) if kc else []
    wr_rest = out_copies(kc, nb)

    gcp = pltpu.make_async_copy(g_hbm, gbuf, wsem.at[0])
    bcp = pltpu.make_async_copy(b_hbm, bbuf, wsem.at[0])

    gcp.start()
    bcp.start()
    rds[0].start()
    rds[1].start()

    pre = {}
    first = 0
    for n, cnt in enumerate(read_chunks):
        pre[first] = [rds[n].wait, rds[n + 2].start]
        first += cnt
    pre.setdefault(0, []).extend([gcp.wait, bcp.wait])
    pre.setdefault(kc, []).extend([rds[-2].wait] + [w.start for w in wr_first])
    pre.setdefault(nb - 1, []).append(rds[-1].wait)

    def body(i, carry):
        for k, ev in pre.items():
            @pl.when(i == k)
            def _(ev=ev):
                for act in ev:
                    act()

        s = pl.multiple_of(i * hw, hw)
        for j in range(ng):
            cols = pl.ds(j * _LANES, _LANES)
            x = xbuf[pl.ds(s, hw), cols].astype(jnp.float32)
            mu = jnp.sum(x, axis=0, keepdims=True) * (1.0 / hw)
            xc = x - mu
            var = jnp.sum(xc * xc, axis=0, keepdims=True) * (1.0 / hw)
            scale = jax.lax.rsqrt(var + _EPS) * gbuf[j:j + 1, :].astype(jnp.float32)
            y = xc * scale + bbuf[j:j + 1, :].astype(jnp.float32)
            obuf[i, :, cols] = y.astype(obuf.dtype)
        return carry

    jax.lax.fori_loop(0, nb, body, 0)
    for w in wr_rest:
        w.start()
    for w in wr_first + wr_rest:
        w.wait()


@jax.jit
def pallas_standalone__instancenorm__sampling_kernel(
    x: jax.Array,
    g: jax.Array,
    b: jax.Array,
):
    B, C, H, W = x.shape
    HW = H * W
    assert C % _LANES == 0 and HW % 32 == 0

    xt = jnp.transpose(x, (0, 2, 3, 1)).reshape(B * HW, C)
    g2 = g.reshape(C // _LANES, _LANES)
    b2 = b.reshape(C // _LANES, _LANES)

    out = pl.pallas_call(
        functools.partial(_kernel, read_chunks=_read_chunks(B // 2), tail=HW // 2),
        in_specs=[pl.BlockSpec(memory_space=pl.ANY)] * 3,
        out_specs=pl.BlockSpec(memory_space=pl.ANY),
        out_shape=jax.ShapeDtypeStruct((B, HW, C), x.dtype),
        scratch_shapes=[
            pltpu.VMEM((B * HW, C), x.dtype),
            pltpu.VMEM((B, HW, C), x.dtype),
            pltpu.VMEM((C // _LANES, _LANES), g.dtype),
            pltpu.VMEM((C // _LANES, _LANES), b.dtype),
            pltpu.SemaphoreType.DMA((2,)),
            pltpu.SemaphoreType.DMA((1,)),
        ],
        compiler_params=pltpu.CompilerParams(vmem_limit_bytes=48 * 1024 * 1024),
    )(xt, g2, b2)
    return jnp.transpose(out.reshape(B, H, W, C), (0, 3, 1, 2))
```
